```python
import jax
import jax.numpy as jnp

def _softmax(x, axis=-1):
    return jax.nn.softmax(x, axis=axis)
def _gelu(x):
    return jax.nn.gelu(x, approximate=True)
def _silu(x):
    return jax.nn.silu(x)
def _sigmoid(x):
    return jax.nn.sigmoid(x)
def _layernorm(x, axis=-1, eps=1e-5):
    m = jnp.mean(x, axis=axis, keepdims=True)
    v = jnp.var(x, axis=axis, keepdims=True)
    return (x - m) / jnp.sqrt(v + eps)
def _scatter_add(tgt, idx, src, axis=0):
    return tgt.at[idx].add(src)
def _segment_sum(src, seg, n):
    return jax.ops.segment_sum(src, seg, n)
class _Rng:
    def __init__(self, key):
        self._k = key
    def _next(self):
        self._k, sub = jax.random.split(self._k)
        return sub
    def normal(self, shape):
        return jax.random.normal(self._next(), shape, dtype=jnp.bfloat16)
    def randint(self, lo, hi, shape):
        return jax.random.randint(self._next(), shape, lo, hi, dtype=jnp.int32)
    def uniform(self, shape, lo=0.0, hi=1.0):
        return jax.random.uniform(self._next(), shape, jnp.bfloat16, lo, hi)
    def permutation(self, n):
        return jax.random.permutation(self._next(), n)


kernel_name = 'interleave_layers__ssm_conv_h3__mixer_s_mlp__prompt'

def setup_inputs():
    _rng = _Rng(jax.random.key(int.from_bytes(__import__("os").urandom(4), "little")))
    _w = (lambda a: (lambda t: t.astype(jnp.bfloat16) if jnp.issubdtype(t.dtype, jnp.floating) else t)(jnp.asarray(a)))
    def _A_setup():
        B, S, D = 1, 2048, 1024
        ks = 4
        return {
            "q": _w((lambda *s: _rng.normal(s) * 0.05)(B, S, D)),
            "k": _w((lambda *s: _rng.normal(s) * 0.05)(B, S, D)),
            "v": _w((lambda *s: _rng.normal(s) * 0.05)(B, S, D)),
            "shift_k": _w((lambda *s: _rng.normal(s) * 0.05)(D, ks) * 0.5),
            "ssm_k": _w((lambda *s: _rng.normal(s) * 0.05)(D, S) * (1.0 / S ** 0.5)),
            "ssm_D": _w((lambda *s: _rng.normal(s) * 0.05)(D)),
        }
    _A_in = _A_setup()

    def _B_setup():
        B, S, D, F = 1, 2048, 1024, 3584
        return {
            "x":  _w((lambda *s: _rng.normal(s) * 0.05)(B, S, D)),
            "w1": _w((lambda *s: _rng.normal(s) * 0.05)(D, D) * (D ** -0.5)),
            "w2": _w((lambda *s: _rng.normal(s) * 0.05)(D, D) * (D ** -0.5)),
            "w3": _w((lambda *s: _rng.normal(s) * 0.05)(D, F) * (D ** -0.5)),
            "w4": _w((lambda *s: _rng.normal(s) * 0.05)(F, D) * (F ** -0.5)),
        }
    _B_in = _B_setup()

    return {
        "A_q": _A_in["q"],
        "A_k": _A_in["k"],
        "A_v": _A_in["v"],
        "A_shift_k": _A_in["shift_k"],
        "A_ssm_k": _A_in["ssm_k"],
        "A_ssm_D": _A_in["ssm_D"],
        "B_x": _B_in["x"],
        "B_w1": _B_in["w1"],
        "B_w2": _B_in["w2"],
        "B_w3": _B_in["w3"],
        "B_w4": _B_in["w4"],
    }

def reference(A_q, A_k, A_v, A_shift_k, A_ssm_k, A_ssm_D, B_x, B_w1, B_w2, B_w3, B_w4):
    def _A_ref(q, k, v, shift_k, ssm_k, ssm_D):
        B, S, D = q.shape
        ks = shift_k.shape[-1]
        k_pad = jnp.pad(k, ((0, 0), (ks - 1, 0), (0, 0)))
        k_shift = jnp.zeros_like(k)
        for t in range(ks):
            k_shift = k_shift + k_pad[:, t:t + S, :] * shift_k[:, ks - 1 - t][None, None, :]
        kv = k_shift * v
        L = 2 * S
        kv_pad = jnp.pad(kv, ((0, 0), (0, S), (0, 0)))
        kf_pad = jnp.pad(ssm_k, ((0, 0), (0, S)))
        kv_f = (lambda x, axes=(-2,-1): jnp.fft.rfft2(x.astype(jnp.float32), axes=axes))(kv_pad[:, None, :, :], axes=(1, 2))
        kf_f = (lambda x, axes=(-2,-1): jnp.fft.rfft2(x.astype(jnp.float32), axes=axes))(kf_pad[:, None, :], axes=(1, 2))
        kf_f = (lambda x, *d: x.transpose(*d))(kf_f, 1, 2, 0)
        y_f = kv_f * kf_f[None, :, :, :]
        y = (lambda x, s, axes=(-2,-1): jnp.fft.irfft2(x, s=s, axes=axes).astype(jnp.bfloat16))(y_f, (1, L), axes=(1, 2))[:, 0, :S, :]
        y = y + kv * ssm_D[None, None, :]
        return q * y

    def _B_ref(x, w1, w2, w3, w4):
        B, S, D = x.shape
        h = _gelu(_layernorm(x, axis=-1) @ w1)
        c = D // 4
        g0 = jnp.pad(h[:, :, 0*c:1*c], ((0, 0), (1, 0), (0, 0)))[:, :S, :]
        g1 = jnp.pad(h[:, :, 1*c:2*c], ((0, 0), (0, 1), (0, 0)))[:, 1:, :]
        g2 = jnp.pad(h[:, :, 2*c:3*c], ((0, 0), (2, 0), (0, 0)))[:, :S, :]
        g3 = jnp.pad(h[:, :, 3*c:   ], ((0, 0), (0, 2), (0, 0)))[:, 2:, :]
        hs = jnp.concatenate([g0, g1, g2, g3], axis=-1) @ w2
        x1 = x + hs
        h2 = _gelu(_layernorm(x1, axis=-1) @ w3) @ w4
        return x1 + h2

    x = A_q
    x = x + _A_ref(_layernorm(x, axis=-1), A_k, A_v, A_shift_k, A_ssm_k, A_ssm_D)
    x = x + _B_ref(_layernorm(x, axis=-1), B_w1, B_w2, B_w3, B_w4)
    x = x + _A_ref(_layernorm(x, axis=-1), A_k, A_v, A_shift_k, A_ssm_k, A_ssm_D)
    x = x + _B_ref(_layernorm(x, axis=-1), B_w1, B_w2, B_w3, B_w4)
    return x
```

```python
import functools
import math

import numpy as np
import jax
import jax.numpy as jnp
from jax import lax
import jax.experimental.pallas as pl
import jax.experimental.pallas.tpu as pltpu

S, D, F = 2048, 1024, 3584
KS = 4
C = 128
NCH = S // C
CB = 128
EPS = 1e-5
PAD = 8


def _dft_mats():
    n = 2 * C
    t = np.arange(C)[:, None].astype(np.float64)
    k = np.arange(C)[None, :].astype(np.float64) + 0.5
    ang = 2.0 * np.pi * t * k / n
    fwd, inv = [], []
    for r in range(4):
        a = ang + 2.0 * np.pi * (r * C) * k / n
        fwd.append(np.concatenate([np.cos(a), -np.sin(a)], axis=1))
        inv.append(np.concatenate([np.cos(a).T, -np.sin(a).T], axis=0) / C)
    return np.stack(fwd).astype(np.float32), np.stack(inv).astype(np.float32)


_FWD, _INV = _dft_mats()


def _ln(x):
    m = jnp.mean(x, axis=-1, keepdims=True)
    xc = x - m
    v = jnp.mean(xc * xc, axis=-1, keepdims=True)
    return xc * lax.rsqrt(v + EPS)


def _gelu(x):
    c = math.sqrt(2.0 / math.pi)
    inner = x * (c + (c * 0.044715) * (x * x))
    hx = 0.5 * x
    return hx + hx * jnp.tanh(inner)


def _kernel(q_hbm, k_hbm, v_hbm, sk_ref, ssmk_hbm, d_ref, w1_hbm, w2_hbm, w3_hbm, w4_hbm,
            fwd_ref, inv_ref, zero_s, o_hbm,
            q_v, k_v, v_v, ssmk_v, w1_v, w2_v, w3_v, w4_v,
            xy_s, z_s, h_all, n_s, nn_s, n1_s, xo_s, u_s, kpad_s, xf0, xf1, kf0, kf1, ws0, ws1, kd0, kd1, o_v, sk_s, sems, osems,
            *, TM, FC, AHEAD, BI, RB_, NB_, SKIPA, PV, LV, DEP, NBP, PEEL):
    f32, bf16 = jnp.float32, jnp.bfloat16
    NCB = D // CB
    NT = S // TM
    xf_s, kf_s, w_s, kd_s = (xf0, xf1), (kf0, kf1), (ws0, ws1), (kd0, kd1)
    yy_s, x_s = xy_s.at[pl.ds(0, S), :], xy_s.at[pl.ds(S, S), :]
    h0_s, h1_s = h_all.at[0], h_all.at[1]

    def a_copies(cb):
        sl = pl.ds(cb * CB if isinstance(cb, int) else pl.multiple_of(cb * CB, CB), CB)
        return (pltpu.make_async_copy(k_hbm.at[:, sl], k_v.at[cb], sems.at[3 * cb]),
                pltpu.make_async_copy(v_hbm.at[:, sl], v_v.at[cb], sems.at[3 * cb + 1]),
                pltpu.make_async_copy(ssmk_hbm.at[sl, :], ssmk_v.at[cb], sems.at[3 * cb + 2]))

    q_cp, w1_cp, w2_cp, w3_cp, w4_cp = [
        pltpu.make_async_copy(src, dst, sems.at[3 * NCB + i])
        for i, (src, dst) in enumerate(((q_hbm, q_v), (w1_hbm, w1_v), (w2_hbm, w2_v), (w3_hbm, w3_v), (w4_hbm, w4_v)))]
    for cb in range(0 if SKIPA else AHEAD):
        for cp in a_copies(cb):
            cp.start()

    sk_t = sk_ref[...].astype(f32)
    d_row = d_ref[...].astype(f32).reshape(1, D)
    for cb in range(NCB):
        sk_s[cb, 0:KS, :] = sk_t[:, cb * CB:(cb + 1) * CB]
        sk_s[cb, KS:KS + 1, :] = d_row[:, cb * CB:(cb + 1) * CB]

    zero8 = jnp.zeros((PAD, D), f32)
    h0_s[pl.ds(0, PAD), :] = zero8
    h0_s[pl.ds(PAD + S, PAD), :] = zero8
    h1_s[pl.ds(0, PAD), :] = zero8
    h1_s[pl.ds(PAD + S, PAD), :] = zero8
    kpad_s[pl.ds(0, PAD), :] = jnp.zeros((PAD, CB), f32)


    def fwd_prep(cb):
        prm = sk_s[cb, 0:KS + 1, :]
        kpad_s[pl.ds(PAD, S), :] = k_v[cb].astype(f32)
        return prm

    def fwd_chunk(cb, p, j, prm):
        ksh = kpad_s[pl.ds(PAD + j * C, C), :] * prm[0:1, :]
        for t in range(1, KS):
            ksh = ksh + kpad_s[pl.ds(PAD + j * C - t, C), :] * prm[t:t + 1, :]
        kv = ksh * v_v[cb, j * C:(j + 1) * C, :].astype(f32)
        kd_s[p][j * C:(j + 1) * C, :] = kv * prm[KS:KS + 1, :]
        x = jnp.dot(kv.T.astype(bf16), fwd_ref[j % 4], preferred_element_type=f32)
        xf_s[p][j, :, 0:2 * C] = x
        xf_s[p][j, :, 2 * C:] = x[:, :C] + x[:, C:]
        kk = jnp.dot(ssmk_v[cb, :, j * C:(j + 1) * C], fwd_ref[j % 4], preferred_element_type=f32)
        kf_s[p][j, :, 0:2 * C] = kk
        kf_s[p][j, :, 2 * C:] = kk[:, :C] + kk[:, C:]

    def prod(p, g, i0, zp):
        rows = slice(g * 8, (g + 1) * 8)
        ld = lambda ref, j: [ref[p][j, rows, c * C:(c + 1) * C] for c in range(3)]
        kc = {}
        acc = {}
        for j in range(i0 + BI):
            x = ld(xf_s, j)
            for i in range(max(i0, j), i0 + BI):
                if i - j not in kc:
                    kc[i - j] = ld(kf_s, i - j)
                pr = [a * b for a, b in zip(x, kc[i - j])]
                acc[i] = pr if i not in acc else [a + b for a, b in zip(acc[i], pr)]
            if j >= i0:
                s1, s2, s3 = acc.pop(j)
                z = (s1 - s2, s3 - s1 - s2)
                w = [a + b for a, b in zip(z, zp)] if j else z
                zp[:] = z
                w_s[p][j, rows, 0:C] = w[0]
                w_s[p][j, rows, C:2 * C] = w[1]

    def inv_chunk(cb, p, i):
        yt = jnp.dot(w_s[p][i].astype(bf16), inv_ref[i % 4], preferred_element_type=f32)
        c0 = cb * CB if isinstance(cb, int) else pl.multiple_of(cb * CB, CB)
        yy_s[i * C:(i + 1) * C, pl.ds(c0, CB)] = kd_s[p][i * C:(i + 1) * C, :] + yt.T

    def conv_step(step, p, do_f, do_p, do_i):
        if do_f:
            for cp in a_copies(step):
                cp.wait()
            if isinstance(step, int) and step == 0:
                for cb in range(AHEAD, NCB):
                    for cp in a_copies(cb):
                        cp.start()
            prm = fwd_prep(step)
        for g in range(NCH):
            if do_i:
                inv_chunk(step - 2, p, g)
            if do_f:
                fwd_chunk(step, p, g, prm)
            if do_p:
                zp = []
                for i0 in range(0, NCH, BI):
                    prod(1 - p, g, i0, zp)

    if not SKIPA:
        conv_step(0, 0, True, False, False)
        q_cp.start()
        w1_cp.start()
        conv_step(1, 1, True, True, False)
        w2_cp.start()
        w3_cp.start()
        w4_cp.start()

        def conv_pair(it, carry):
            conv_step(2 * it, 0, True, True, True)
            conv_step(2 * it + 1, 1, True, True, True)
            return carry

        lax.fori_loop(1, NCB // 2, conv_pair, 0)
        conv_step(NCB, 0, False, True, True)
        conv_step(NCB + 1, 1, False, False, True)
    else:
        for cp in (q_cp, w1_cp, w2_cp, w3_cp, w4_cp):
            cp.start()

    def tile(t):
        return t * TM if isinstance(t, int) else pl.multiple_of(t * TM, TM)

    zero = zero_s[0]
    RB = RB_
    NR = TM // RB
    NB = NB_

    def weave(main, side):
        mo, so = [], []
        for i, f in enumerate(main):
            mo.append(f())
            so += [g() for g in side[len(side) * i // len(main):len(side) * (i + 1) // len(main)]]
        return mo, so

    def gate_tasks(load, r0):
        pend = []

        def task(i):
            rows = pl.ds(r0 + i * RB, RB)
            x = load(i)
            x = x + _ln(x) * xy_s[pl.ds(pl.multiple_of(r0 + i * RB + zero, RB), RB), :]
            z = _ln(x)
            xy_s[pl.ds(S + r0 + i * RB, RB), :] = x
            z_s[rows, :] = z
            n = _ln(z)
            pend.append(n[RB - 8:, D - 128:])
            if len(pend) > DEP:
                xy_s[pl.ds(2 * S, 8), 0:128] = pend.pop(0)
            return n.astype(bf16)
        return [functools.partial(task, i) for i in range(NR)]

    def proj1_tasks(n, r0, h_s):
        def task(j):
            cols = slice(j * NB, (j + 1) * NB)
            h_s[pl.ds(r0 + PAD, TM), cols] = _gelu(jnp.dot(n, w1_v[:, cols], preferred_element_type=f32))
        return [functools.partial(task, j) for j in range(D // NB)]

    def first_gate_tasks(t):
        r0 = tile(t)
        return gate_tasks(lambda i: q_v[pl.ds(r0 + i * RB, RB), :].astype(f32), r0)

    def head_tasks(r0, h_s):
        c = D // 4
        hv = h_s.at[pl.ds(r0, TM + 2 * PAD), :]
        g = jnp.concatenate([hv[pl.ds(PAD + o, TM), i * c:(i + 1) * c] for i, o in enumerate((-1, 1, -2, 2))],
                            axis=1).astype(bf16)

        def task(j):
            cols = slice(j * NB, (j + 1) * NB)
            u_s[:, cols] = z_s[pl.ds(r0, TM), cols] + jnp.dot(g, w2_v[:, cols], preferred_element_type=f32)
        return [functools.partial(task, j) for j in range(D // NB)]

    def head_norm_tasks():
        def task(i):
            rows = slice(i * RB, (i + 1) * RB)
            n_s[rows, :] = _ln(u_s[rows, :]).astype(bf16)
        return [functools.partial(task, i) for i in range(NR)]

    def ffn_tasks(r0, box):
        n = n_s[...]
        box.append(x_s[pl.ds(r0, TM), :] + u_s[...])

        def task(fc):
            a = jnp.dot(n, w3_v[:, fc * FC:(fc + 1) * FC], preferred_element_type=f32)
            box[0] = box[0] + jnp.dot(_gelu(a).astype(bf16), w4_v[fc * FC:(fc + 1) * FC, :],
                                      preferred_element_type=f32)
        return [functools.partial(task, fc) for fc in range(F // FC)]

    def run(tasks):
        return [f() for f in tasks]

    def first(t, carry):
        n = n_s[...]
        if PV == 0:
            run(proj1_tasks(n, tile(t), h0_s))
            n_s[...] = jnp.concatenate(run(first_gate_tasks(jnp.minimum(t + 1, NT - 1))), axis=0)
        elif PV == 1:
            n2 = jnp.concatenate(run(first_gate_tasks(jnp.minimum(t + 1, NT - 1))), axis=0)
            run(proj1_tasks(n, tile(t), h0_s))
            n_s[...] = n2
        elif PV == 2:
            _, n2 = weave(proj1_tasks(n, tile(t), h0_s), first_gate_tasks(jnp.minimum(t + 1, NT - 1)))
            n_s[...] = jnp.concatenate(n2, axis=0)
        elif PV == 3:
            n_s[...] = jnp.concatenate(run(first_gate_tasks(jnp.minimum(t + 1, NT - 1))), axis=0)
            run(proj1_tasks(n, tile(t), h0_s))
        elif PV == 5:
            t1 = jnp.minimum(t + 1, NT - 1)
            src = pl.multiple_of((t % 2) * TM, TM)
            dst = pl.multiple_of(((t + 1) % 2) * TM, TM)

            def dot_task(j):
                cols = slice(j * NBP, (j + 1) * NBP)
                h0_s[pl.ds(tile(t) + PAD, TM), cols] = _gelu(
                    jnp.dot(nn_s[pl.ds(src, TM), :], w1_v[:, cols], preferred_element_type=f32))

            def keep(i, g):
                nn_s[pl.ds(dst + i * RB, RB), :] = g()

            weave([functools.partial(dot_task, j) for j in range(D // NBP)],
                  [functools.partial(keep, i, g) for i, g in enumerate(first_gate_tasks(t1))])
        elif PV == 4:
            n1 = jnp.concatenate(run(first_gate_tasks(2 * t + 1)), axis=0)
            run(proj1_tasks(n, tile(2 * t), h0_s))
            n_s[...] = jnp.concatenate(run(first_gate_tasks(jnp.minimum(2 * t + 2, NT - 1))), axis=0)
            run(proj1_tasks(n1, tile(2 * t + 1), h0_s))
        return carry

    q_cp.wait()
    n_s[...] = jnp.concatenate(run(first_gate_tasks(0)), axis=0)
    nn_s[0:TM, :] = n_s[...]
    w1_cp.wait()
    lax.fori_loop(0, NT // 2 if PV == 4 else NT, first, 0)
    w2_cp.wait()
    run(head_tasks(0, h0_s))
    run(head_norm_tasks())
    w3_cp.wait()
    w4_cp.wait()

    def layer1(t, carry):
        r0 = tile(t)
        box = []
        hn = lambda: head_tasks(tile((t + 1) % NT), h_all.at[(t + 1) // NT])
        gt = lambda: gate_tasks(lambda i: box[0][i * RB:(i + 1) * RB], r0)
        ft = ffn_tasks(r0, box)
        if LV == 0:
            run(ft)
            run(hn())
            n = run(gt())
            run(head_norm_tasks())
            run(proj1_tasks(jnp.concatenate(n, axis=0), r0, h1_s))
        elif LV == 1:
            tp = jnp.maximum(t - 1, 0)
            run(proj1_tasks(n1_s[...], tile(tp), h1_s))
            run(ft)
            run(hn())
            run(head_norm_tasks())
            n1_s[...] = jnp.concatenate(run(gt()), axis=0)
        elif LV == 2:
            run(ft[:-1])
            run(hn())
            run(ft[-1:])
            run(head_norm_tasks())
            n = run(gt())
            run(proj1_tasks(jnp.concatenate(n, axis=0), r0, h1_s))
        elif LV == 3:
            tp = tile(jnp.maximum(t - 1, 0))
            n = run(gate_tasks(lambda i: xo_s[i * RB:(i + 1) * RB, :], tp))
            run(ft[:2])
            run(proj1_tasks(jnp.concatenate(n, axis=0), tp, h1_s))
            run(ft[2:-1])
            run(hn())
            run(ft[-1:])
            run(head_norm_tasks())
            xo_s[...] = box[0]
        return carry

    lax.fori_loop(0, NT, layer1, 0)

    def out_copy(t):
        rows = pl.ds(tile(t), TM)
        return pltpu.make_async_copy(o_v.at[rows, :], o_hbm.at[rows, :], osems.at[t])

    def layer2(t, carry, last=False):
        box = []
        tasks = ffn_tasks(tile(t), box)
        run(tasks[:-1])
        if not last:
            run(head_tasks(tile(t + 1 if PEEL else jnp.minimum(t + 1, NT - 1)), h1_s))
        run(tasks[-1:])
        if not last:
            run(head_norm_tasks())
        o_v[pl.ds(tile(t), TM), :] = box[0].astype(bf16)
        out_copy(t).start()
        return carry

    lax.fori_loop(0, NT - PEEL, layer2, 0)
    if PEEL:
        layer2(NT - 1, 0, last=True)
    for t in range(NT):
        out_copy(t).wait()


def build(TM=256, FC=512, AHEAD=2, BI=16, RB=16, NB=256, SKIPA=0, PV=5, LV=0, DEP=3, NBP=256, PEEL=1, flags=None):
    f32, bf16 = jnp.float32, jnp.bfloat16
    NCB = D // CB
    anyspec = pl.BlockSpec(memory_space=pl.ANY)
    vm = pl.BlockSpec(memory_space=pltpu.VMEM)

    @jax.jit
    def fn(A_q, A_k, A_v, A_shift_k, A_ssm_k, A_ssm_D, B_x, B_w1, B_w2, B_w3, B_w4):
        call = pl.pallas_call(
            functools.partial(_kernel, TM=TM, FC=FC, AHEAD=AHEAD, BI=BI, RB_=RB, NB_=NB, SKIPA=SKIPA, PV=PV, LV=LV, DEP=DEP, NBP=NBP, PEEL=PEEL),
            out_shape=jax.ShapeDtypeStruct((S, D), bf16),
            in_specs=[anyspec, anyspec, anyspec, vm, anyspec, vm, anyspec, anyspec, anyspec, anyspec, vm, vm, pl.BlockSpec(memory_space=pltpu.SMEM)],
            out_specs=anyspec,
            scratch_shapes=[
                pltpu.VMEM((S, D), bf16),
                pltpu.VMEM((NCB, S, CB), bf16),
                pltpu.VMEM((NCB, S, CB), bf16),
                pltpu.VMEM((NCB, CB, S), bf16),
                pltpu.VMEM((D, D), bf16),
                pltpu.VMEM((D, D), bf16),
                pltpu.VMEM((D, F), bf16),
                pltpu.VMEM((F, D), bf16),
                pltpu.VMEM((2 * S + 8, D), f32),
                pltpu.VMEM((S, D), f32),
                pltpu.VMEM((2, S + 2 * PAD, D), f32),
                pltpu.VMEM((TM, D), bf16), pltpu.VMEM((2 * TM, D), bf16), pltpu.VMEM((TM, D), bf16), pltpu.VMEM((TM, D), f32),
                pltpu.VMEM((TM, D), f32),
                pltpu.VMEM((S + PAD, CB), f32),
                *[pltpu.VMEM((NCH, CB, 3 * C), f32)] * 4,
                *[pltpu.VMEM((NCH, CB, 2 * C), f32)] * 2,
                *[pltpu.VMEM((S, CB), f32)] * 2,
                pltpu.VMEM((S, D), bf16),
                pltpu.VMEM((NCB, 8, CB), f32),
                pltpu.SemaphoreType.DMA((3 * NCB + 5,)),
                pltpu.SemaphoreType.DMA((S // TM,)),
            ],
            compiler_params=pltpu.CompilerParams(vmem_limit_bytes=120 * 1024 * 1024, flags=flags),
        )
        out = call(A_q.reshape(S, D), A_k.reshape(S, D), A_v.reshape(S, D), A_shift_k.T, A_ssm_k, A_ssm_D,
                   B_w1, B_w2, B_w3, B_w4, _FWD.astype(bf16), _INV.astype(bf16), np.zeros((1,), np.int32))
        return out.reshape(1, S, D)

    return fn


_impl = build()


@jax.jit
def pallas_interleave_layers__ssm_conv_h3__mixer_s_mlp__prompt_kernel(
        A_q, A_k, A_v, A_shift_k, A_ssm_k, A_ssm_D, B_x, B_w1, B_w2, B_w3, B_w4):
    return _impl(A_q, A_k, A_v, A_shift_k, A_ssm_k, A_ssm_D, B_x, B_w1, B_w2, B_w3, B_w4)
```

```python
import math

import numpy as np
import jax
import jax.numpy as jnp
from jax import lax
import jax.experimental.pallas as pl
import jax.experimental.pallas.tpu as pltpu

S, D, F = 2048, 1024, 3584
KS = 4
C = 128
NCH = S // C
CB = 128
NCB = D // CB
TM = 256
NT = S // TM
FC = 512
NB = 256
RB = 16
NR = TM // RB
PAD = 8
AHEAD = 2
EPS = 1e-5


def _dft_mats():
    n = 2 * C
    t = np.arange(C)[:, None].astype(np.float64)
    k = np.arange(C)[None, :].astype(np.float64) + 0.5
    fwd, inv = [], []
    for r in range(4):
        a = 2.0 * np.pi * (t + r * C) * k / n
        fwd.append(np.concatenate([np.cos(a), -np.sin(a)], axis=1))
        inv.append(np.concatenate([np.cos(a).T, -np.sin(a).T], axis=0) / C)
    return np.stack(fwd).astype(np.float32), np.stack(inv).astype(np.float32)


_FWD, _INV = _dft_mats()


def _ln(x):
    m = jnp.mean(x, axis=-1, keepdims=True)
    xc = x - m
    v = jnp.mean(xc * xc, axis=-1, keepdims=True)
    return xc * lax.rsqrt(v + EPS)


def _gelu(x):
    c = math.sqrt(2.0 / math.pi)
    inner = x * (c + (c * 0.044715) * (x * x))
    hx = 0.5 * x
    return hx + hx * jnp.tanh(inner)


def _aligned(i, m):
    return i if isinstance(i, int) else pl.multiple_of(i, m)


def _kernel(q_hbm, k_hbm, v_hbm, sk_ref, ssmk_hbm, d_ref, w1_hbm, w2_hbm, w3_hbm, w4_hbm,
            fwd_ref, inv_ref, zero_ref, o_hbm,
            q_v, k_v, v_v, ssmk_v, w1_v, w2_v, w3_v, w4_v, o_v,
            yy_s, x_s, z_s, h_all, n_s, u_s,
            kpad_s, xf0, xf1, kf0, kf1, ws0, ws1, kd0, kd1, sk_s, sems, osems):
    f32, bf16 = jnp.float32, jnp.bfloat16
    xf_s, kf_s, w_s, kd_s = (xf0, xf1), (kf0, kf1), (ws0, ws1), (kd0, kd1)
    h0_s, h1_s = h_all.at[0], h_all.at[1]

    def dot(a, b):
        return jnp.dot(a, b, preferred_element_type=f32)

    def conv_copies(cb):
        sl = pl.ds(_aligned(cb * CB, CB), CB)
        return (pltpu.make_async_copy(ssmk_hbm.at[sl, :], ssmk_v.at[cb], sems.at[3 * cb]),
                pltpu.make_async_copy(k_hbm.at[:, sl], k_v.at[cb], sems.at[3 * cb + 1]),
                pltpu.make_async_copy(v_hbm.at[:, sl], v_v.at[cb], sems.at[3 * cb + 2]))

    q_cp, w1_cp, w2_cp, w3_cp, w4_cp = [
        pltpu.make_async_copy(src, dst, sems.at[3 * NCB + i])
        for i, (src, dst) in enumerate(
            ((q_hbm, q_v), (w1_hbm, w1_v), (w2_hbm, w2_v), (w3_hbm, w3_v), (w4_hbm, w4_v)))]
    for cb in range(AHEAD):
        for cp in conv_copies(cb):
            cp.start()

    taps = sk_ref[...].astype(f32)
    gain = d_ref[...].astype(f32).reshape(1, D)
    for cb in range(NCB):
        sk_s[cb, 0:KS, :] = taps[:, cb * CB:(cb + 1) * CB]
        sk_s[cb, KS:KS + 1, :] = gain[:, cb * CB:(cb + 1) * CB]
    for h_s in (h0_s, h1_s):
        h_s[pl.ds(0, PAD), :] = jnp.zeros((PAD, D), f32)
        h_s[pl.ds(PAD + S, PAD), :] = jnp.zeros((PAD, D), f32)
    kpad_s[pl.ds(0, PAD), :] = jnp.zeros((PAD, CB), f32)

    zero = zero_ref[0]
    never8 = (jnp.zeros((8, 128), jnp.int32) + zero) != 0
    never_rb = (jnp.zeros((RB, 128), jnp.int32) + zero) != 0

    def kv_chunk(cb, p, j, prm):
        ksh = kpad_s[pl.ds(PAD + j * C, C), :] * prm[0:1, :]
        for t in range(1, KS):
            ksh = ksh + kpad_s[pl.ds(PAD + j * C - t, C), :] * prm[t:t + 1, :]
        kv = ksh * v_v[cb, j * C:(j + 1) * C, :].astype(f32)
        kd_s[p][j * C:(j + 1) * C, :] = kv * prm[KS:KS + 1, :]
        return kv.astype(bf16).T

    def spectra(ref, js, chunks):
        r = dot(jnp.concatenate(chunks, axis=0), fwd_ref[js[0] % 4])
        for n, j in enumerate(js):
            x = r[n * CB:(n + 1) * CB]
            ref[j, :, 0:2 * C] = x
            ref[j, :, 2 * C:] = x[:, :C] + x[:, C:]
        return [r[m * 8:(m + 1) * 8, C:] for m in range(r.shape[0] // 8)]

    def filter_spectra(cb, p, js):
        return spectra(kf_s[p], js, [ssmk_v[cb, :, j * C:(j + 1) * C] for j in js])

    def products(p, g, ties):
        rows = slice(g * 8, (g + 1) * 8)
        load = lambda ref, j: [ref[p][j, rows, c * C:(c + 1) * C] for c in range(3)]
        kf, acc, prev = {}, {}, None
        for j in range(NCH):
            x = load(xf_s, j)
            if ties[j] is not None:
                x[0] = jnp.where(never8, ties[j], x[0])
            for i in range(j, NCH):
                if i - j not in kf:
                    kf[i - j] = load(kf_s, i - j)
                pr = [a * b for a, b in zip(x, kf[i - j])]
                acc[i] = pr if i not in acc else [a + b for a, b in zip(acc[i], pr)]
            s1, s2, s3 = acc.pop(j)
            z = (s1 - s2, s3 - s1 - s2)
            w = z if prev is None else (z[0] + prev[0], z[1] + prev[1])
            prev = z
            w_s[p][j, rows, 0:C] = w[0]
            w_s[p][j, rows, C:2 * C] = w[1]

    def inverse(cb, p, js):
        r = dot(jnp.concatenate([w_s[p][i].astype(bf16) for i in js], axis=0), inv_ref[js[0] % 4])
        cols = pl.ds(_aligned(cb * CB, CB), CB)
        for n, i in enumerate(js):
            yy_s[i * C:(i + 1) * C, cols] = kd_s[p][i * C:(i + 1) * C, :] + r[n * CB:(n + 1) * CB].T
        return [r[m * 8:(m + 1) * 8, :] for m in range(r.shape[0] // 8)]

    groups = [[4 * n + r for n in range(4)] for r in range(4)]
    J0 = 8

    def conv_step(step, p, do_fwd, do_prod, do_inv):
        first = isinstance(step, int) and step == 0
        if do_fwd:
            f_cp, k_cp, v_cp = conv_copies(step)
            f_cp.wait()
            if first:
                for js in groups:
                    filter_spectra(step, p, js)
            k_cp.wait()
            v_cp.wait()
            if first:
                for cb in range(AHEAD, NCB):
                    for cp in conv_copies(cb):
                        cp.start()
            prm = sk_s[step, 0:KS + 1, :]
            kpad_s[pl.ds(PAD, S), :] = k_v[step].astype(f32)
        for r, js in enumerate(groups):
            done = []
            if do_inv:
                done += inverse(step - 2, p, js)
            if do_fwd:
                done += spectra(xf_s[p], js, [kv_chunk(step, p, j, prm) for j in js])
                if not first:
                    done += filter_spectra(step, p, js)
            if do_prod:
                per = len(done) // 4
                total = sum(NCH - j for j in range(J0, NCH))
                for n in range(4):
                    ties = [None] * NCH
                    for j in range(J0, NCH):
                        frac = sum(NCH - jj for jj in range(J0, j + 1)) / total
                        ties[j] = done[n * per + min(int(frac * per), per - 1)]
                    products(1 - p, 4 * r + n, ties)

    conv_step(0, 0, True, False, False)
    q_cp.start()
    w1_cp.start()
    conv_step(1, 1, True, True, False)
    w2_cp.start()
    w3_cp.start()
    w4_cp.start()

    def conv_pair(it, carry):
        conv_step(2 * it, 0, True, True, True)
        conv_step(2 * it + 1, 1, True, True, True)
        return carry

    lax.fori_loop(1, NCB // 2, conv_pair, 0)
    conv_step(NCB, 0, False, True, True)
    conv_step(NCB + 1, 1, False, False, True)

    def tile(t):
        return _aligned(t * TM, TM)

    def pieces(results, count, lo, hi):
        ps = [r[m * RB:(m + 1) * RB, c:c + 128]
              for r in results for c in range(0, r.shape[1], 128) for m in range(NR)]
        return [ps[int(len(ps) * (lo + (hi - lo) * k / count))] for k in range(count)]

    def after(x, tie):
        if tie is None:
            return x
        return jnp.concatenate([jnp.where(never_rb, tie, x[:, :128]), x[:, 128:]], axis=1)

    def gate(load, r0, along=None, hi=None):
        skew = 2
        ties = pieces(along, NR + 2 * skew, 0.0, hi) if along else [None] * (NR + 2 * skew)
        out = []
        for i in range(NR):
            rows = pl.ds(r0 + i * RB, RB)
            x = after(load(i), ties[i])
            x = x + _ln(x) * yy_s[rows, :]
            z = _ln(after(x, ties[i + skew]))
            x_s[rows, :] = x
            z_s[rows, :] = z
            out.append(_ln(after(z, ties[i + 2 * skew])).astype(bf16))
        return jnp.concatenate(out, axis=0)

    def first_gate(t, along=None):
        r0 = tile(t)
        return gate(lambda i: q_v[pl.ds(r0 + i * RB, RB), :].astype(f32), r0, along, 0.6)

    def token_in(n, r0, h_s):
        res = []
        for j in range(D // NB):
            cols = slice(j * NB, (j + 1) * NB)
            res.append(dot(n, w1_v[:, cols]))
            h_s[pl.ds(r0 + PAD, TM), cols] = _gelu(res[-1])
        return res

    def token_out(r0, h_s):
        c = D // 4
        hv = h_s.at[pl.ds(r0, TM + 2 * PAD), :]
        g = jnp.concatenate([hv[pl.ds(PAD + o, TM), i * c:(i + 1) * c]
                             for i, o in enumerate((-1, 1, -2, 2))], axis=1).astype(bf16)
        res = []
        for j in range(D // NB):
            cols = slice(j * NB, (j + 1) * NB)
            res.append(z_s[pl.ds(r0, TM), cols] + dot(g, w2_v[:, cols]))
            u_s[:, cols] = res[-1]
        return res

    def channel_norm(ties=None):
        for i in range(NR):
            rows = slice(i * RB, (i + 1) * RB)
            n_s[rows, :] = _ln(after(u_s[rows, :], ties[i] if ties else None)).astype(bf16)

    def hidden(n, fc):
        return _gelu(dot(n, w3_v[:, fc * FC:(fc + 1) * FC])).astype(bf16)

    def channel_mlp(n, acc, fcs):
        for fc in fcs:
            acc = acc + dot(hidden(n, fc), w4_v[fc * FC:(fc + 1) * FC, :])
        return acc

    NF = F // FC

    def prologue(t, carry):
        res = token_in(n_s[...], tile(t), h0_s)
        n_s[...] = first_gate(jnp.minimum(t + 1, NT - 1), res)
        return carry

    q_cp.wait()
    n_s[...] = first_gate(0)
    w1_cp.wait()
    lax.fori_loop(0, NT, prologue, 0)
    w2_cp.wait()
    token_out(0, h0_s)
    channel_norm()
    w3_cp.wait()
    w4_cp.wait()

    def layer1(t, carry):
        r0 = tile(t)
        x = channel_mlp(n_s[...], x_s[pl.ds(r0, TM), :] + u_s[...], range(NF))
        res = token_out(tile((t + 1) % NT), h_all.at[(t + 1) // NT])
        n = gate(lambda i: x[i * RB:(i + 1) * RB], r0, res, 0.85)
        res = token_in(n, r0, h1_s)
        channel_norm(pieces(res, NR, 0.05, 0.8))
        return carry

    lax.fori_loop(0, NT, layer1, 0)

    def out_copy(t, cols, sem):
        rows = pl.ds(tile(t), TM)
        return pltpu.make_async_copy(o_v.at[rows, cols], o_hbm.at[rows, cols], osems.at[sem])

    def layer2(t, carry):
        r0 = tile(t)
        n = n_s[...]
        x = channel_mlp(n, x_s[pl.ds(r0, TM), :] + u_s[...], range(NF - 1))
        token_out(tile(t + 1), h1_s)
        x = channel_mlp(n, x, [NF - 1])
        channel_norm()
        o_v[pl.ds(r0, TM), :] = x.astype(bf16)
        out_copy(t, slice(0, D), t).start()
        return carry

    lax.fori_loop(0, NT - 1, layer2, 0)

    t = NT - 1
    n = n_s[...]
    x = channel_mlp(n, x_s[pl.ds(tile(t), TM), :] + u_s[...], range(NF - 1))
    a = hidden(n, NF - 1)
    halves = [slice(0, D // 2), slice(D // 2, D)]
    for j, cols in enumerate(halves):
        o_v[pl.ds(tile(t), TM), cols] = (x[:, cols] + dot(a, w4_v[(NF - 1) * FC:, cols])).astype(bf16)
        out_copy(t, cols, t + j).start()
    for tt in range(NT - 1):
        out_copy(tt, slice(0, D), tt).wait()
    for j, cols in enumerate(halves):
        out_copy(t, cols, t + j).wait()


@jax.jit
def pallas_interleave_layers__ssm_conv_h3__mixer_s_mlp__prompt_kernel(
        A_q, A_k, A_v, A_shift_k, A_ssm_k, A_ssm_D, B_x, B_w1, B_w2, B_w3, B_w4):
    del B_x
    f32, bf16 = jnp.float32, jnp.bfloat16
    hbm = pl.BlockSpec(memory_space=pl.ANY)
    vmem = pl.BlockSpec(memory_space=pltpu.VMEM)
    smem = pl.BlockSpec(memory_space=pltpu.SMEM)
    out = pl.pallas_call(
        _kernel,
        out_shape=jax.ShapeDtypeStruct((S, D), bf16),
        in_specs=[hbm, hbm, hbm, vmem, hbm, vmem, hbm, hbm, hbm, hbm, vmem, vmem, smem],
        out_specs=hbm,
        scratch_shapes=[
            pltpu.VMEM((S, D), bf16),
            pltpu.VMEM((NCB, S, CB), bf16),
            pltpu.VMEM((NCB, S, CB), bf16),
            pltpu.VMEM((NCB, CB, S), bf16),
            pltpu.VMEM((D, D), bf16),
            pltpu.VMEM((D, D), bf16),
            pltpu.VMEM((D, F), bf16),
            pltpu.VMEM((F, D), bf16),
            pltpu.VMEM((S, D), bf16),
            pltpu.VMEM((S, D), f32),
            pltpu.VMEM((S, D), f32),
            pltpu.VMEM((S, D), f32),
            pltpu.VMEM((2, S + 2 * PAD, D), f32),
            pltpu.VMEM((TM, D), bf16),
            pltpu.VMEM((TM, D), f32),
            pltpu.VMEM((S + PAD, CB), f32),
            *[pltpu.VMEM((NCH, CB, 3 * C), f32)] * 4,
            *[pltpu.VMEM((NCH, CB, 2 * C), f32)] * 2,
            *[pltpu.VMEM((S, CB), f32)] * 2,
            pltpu.VMEM((NCB, 8, CB), f32),
            pltpu.SemaphoreType.DMA((3 * NCB + 5,)),
            pltpu.SemaphoreType.DMA((NT + 1,)),
        ],
        compiler_params=pltpu.CompilerParams(vmem_limit_bytes=120 * 1024 * 1024),
    )(A_q.reshape(S, D), A_k.reshape(S, D), A_v.reshape(S, D), A_shift_k.T, A_ssm_k, A_ssm_D,
      B_w1, B_w2, B_w3, B_w4, _FWD.astype(bf16), _INV.astype(bf16), np.zeros((1,), np.int32))
    return out.reshape(1, S, D)
```

```python
import math

import numpy as np
import jax
import jax.numpy as jnp
from jax import lax
import jax.experimental.pallas as pl
import jax.experimental.pallas.tpu as pltpu

S, D, F = 2048, 1024, 3584
KS = 4
C = 128
NCH = S // C
CB = 128
NCB = D // CB
TM = 256
NT = S // TM
FC = 512
NB = 256
RB = 16
NR = TM // RB
PAD = 8
AHEAD = 2
EPS = 1e-5


def _dft_mats():
    n = 2 * C
    t = np.arange(C)[:, None].astype(np.float64)
    k = np.arange(C)[None, :].astype(np.float64) + 0.5
    fwd, inv = [], []
    for r in range(4):
        a = 2.0 * np.pi * (t + r * C) * k / n
        fwd.append(np.concatenate([np.cos(a), -np.sin(a)], axis=1))
        inv.append(np.concatenate([np.cos(a).T, -np.sin(a).T], axis=0) / C)
    return np.stack(fwd).astype(np.float32), np.stack(inv).astype(np.float32)


_FWD, _INV = _dft_mats()


def _ln(x):
    m = jnp.mean(x, axis=-1, keepdims=True)
    xc = x - m
    v = jnp.mean(xc * xc, axis=-1, keepdims=True)
    return xc * lax.rsqrt(v + EPS)


def _gelu(x):
    c = math.sqrt(2.0 / math.pi)
    inner = x * (c + (c * 0.044715) * (x * x))
    hx = 0.5 * x
    return hx + hx * jnp.tanh(inner)


def _aligned(i, m):
    return i if isinstance(i, int) else pl.multiple_of(i, m)


def _kernel(q_hbm, k_hbm, v_hbm, sk_ref, ssmk_hbm, d_ref, w1_hbm, w2_hbm, w3_hbm, w4_hbm,
            fwd_ref, inv_ref, zero_ref, o_hbm,
            q_v, k_v, v_v, ssmk_v, w1_v, w2_v, w3_v, w4_v, o_v,
            xy_s, z_s, h_all, n_s, u_s,
            kpad_s, xf0, xf1, kf0, kf1, ws0, ws1, kd0, kd1, sk_s, sems, osems):
    f32, bf16 = jnp.float32, jnp.bfloat16
    xf_s, kf_s, w_s, kd_s = (xf0, xf1), (kf0, kf1), (ws0, ws1), (kd0, kd1)
    h0_s, h1_s = h_all.at[0], h_all.at[1]
    yy_s, x_s = xy_s.at[pl.ds(0, S), :], xy_s.at[pl.ds(S, S), :]

    def dot(a, b):
        return jnp.dot(a, b, preferred_element_type=f32)

    def conv_copies(cb):
        sl = pl.ds(_aligned(cb * CB, CB), CB)
        return (pltpu.make_async_copy(ssmk_hbm.at[sl, :], ssmk_v.at[cb], sems.at[3 * cb]),
                pltpu.make_async_copy(k_hbm.at[:, sl], k_v.at[cb], sems.at[3 * cb + 1]),
                pltpu.make_async_copy(v_hbm.at[:, sl], v_v.at[cb], sems.at[3 * cb + 2]))

    q_cp, w1_cp, w2_cp, w3_cp, w4_cp = [
        pltpu.make_async_copy(src, dst, sems.at[3 * NCB + i])
        for i, (src, dst) in enumerate(
            ((q_hbm, q_v), (w1_hbm, w1_v), (w2_hbm, w2_v), (w3_hbm, w3_v), (w4_hbm, w4_v)))]
    for cb in range(AHEAD):
        for cp in conv_copies(cb):
            cp.start()

    taps = sk_ref[...].astype(f32)
    gain = d_ref[...].astype(f32).reshape(1, D)
    for cb in range(NCB):
        sk_s[cb, 0:KS, :] = taps[:, cb * CB:(cb + 1) * CB]
        sk_s[cb, KS:KS + 1, :] = gain[:, cb * CB:(cb + 1) * CB]
    for h_s in (h0_s, h1_s):
        h_s[pl.ds(0, PAD), :] = jnp.zeros((PAD, D), f32)
        h_s[pl.ds(PAD + S, PAD), :] = jnp.zeros((PAD, D), f32)
    kpad_s[pl.ds(0, PAD), :] = jnp.zeros((PAD, CB), f32)

    zero = zero_ref[0]
    never8 = (jnp.zeros((8, 128), jnp.int32) + zero) != 0
    never_rb = (jnp.zeros((RB, 128), jnp.int32) + zero) != 0

    def kv_chunk(cb, p, j, prm):
        ksh = kpad_s[pl.ds(PAD + j * C, C), :] * prm[0:1, :]
        for t in range(1, KS):
            ksh = ksh + kpad_s[pl.ds(PAD + j * C - t, C), :] * prm[t:t + 1, :]
        kv = ksh * v_v[cb, j * C:(j + 1) * C, :].astype(f32)
        kd_s[p][j * C:(j + 1) * C, :] = kv * prm[KS:KS + 1, :]
        return kv.astype(bf16).T

    def spectra(ref, js, chunks):
        r = dot(jnp.concatenate(chunks, axis=0), fwd_ref[js[0] % 4])
        for n, j in enumerate(js):
            x = r[n * CB:(n + 1) * CB]
            ref[j, :, 0:2 * C] = x
            ref[j, :, 2 * C:] = x[:, :C] + x[:, C:]
        return [r[m * 8:(m + 1) * 8, C:] for m in range(r.shape[0] // 8)]

    def filter_spectra(cb, p, js):
        return spectra(kf_s[p], js, [ssmk_v[cb, :, j * C:(j + 1) * C] for j in js])

    def products(p, g, ties):
        rows = slice(g * 8, (g + 1) * 8)
        load = lambda ref, j: [ref[p][j, rows, c * C:(c + 1) * C] for c in range(3)]
        kf, acc, prev = {}, {}, None
        for j in range(NCH):
            x = load(xf_s, j)
            if ties[j] is not None:
                x[0] = jnp.where(never8, ties[j], x[0])
            for i in range(j, NCH):
                if i - j not in kf:
                    kf[i - j] = load(kf_s, i - j)
                pr = [a * b for a, b in zip(x, kf[i - j])]
                acc[i] = pr if i not in acc else [a + b for a, b in zip(acc[i], pr)]
            s1, s2, s3 = acc.pop(j)
            z = (s1 - s2, s3 - s1 - s2)
            w = z if prev is None else (z[0] + prev[0], z[1] + prev[1])
            prev = z
            w_s[p][j, rows, 0:C] = w[0]
            w_s[p][j, rows, C:2 * C] = w[1]

    def inverse(cb, p, js):
        r = dot(jnp.concatenate([w_s[p][i].astype(bf16) for i in js], axis=0), inv_ref[js[0] % 4])
        cols = pl.ds(_aligned(cb * CB, CB), CB)
        for n, i in enumerate(js):
            yy_s[i * C:(i + 1) * C, cols] = kd_s[p][i * C:(i + 1) * C, :] + r[n * CB:(n + 1) * CB].T
        return [r[m * 8:(m + 1) * 8, :] for m in range(r.shape[0] // 8)]

    groups = [[4 * n + r for n in range(4)] for r in range(4)]
    J0 = 8

    def conv_step(step, p, do_fwd, do_prod, do_inv):
        first = isinstance(step, int) and step == 0
        if do_fwd:
            f_cp, k_cp, v_cp = conv_copies(step)
            f_cp.wait()
            if first:
                for js in groups:
                    filter_spectra(step, p, js)
            k_cp.wait()
            v_cp.wait()
            if first:
                for cb in range(AHEAD, NCB):
                    for cp in conv_copies(cb):
                        cp.start()
            prm = sk_s[step, 0:KS + 1, :]
            kpad_s[pl.ds(PAD, S), :] = k_v[step].astype(f32)
        for r, js in enumerate(groups):
            done = []
            if do_inv:
                done += inverse(step - 2, p, js)
            if do_fwd:
                done += spectra(xf_s[p], js, [kv_chunk(step, p, j, prm) for j in js])
                if not first:
                    done += filter_spectra(step, p, js)
            if do_prod:
                per = len(done) // 4
                total = sum(NCH - j for j in range(J0, NCH))
                for n in range(4):
                    ties = [None] * NCH
                    for j in range(J0, NCH):
                        frac = sum(NCH - jj for jj in range(J0, j + 1)) / total
                        ties[j] = done[n * per + min(int(frac * per), per - 1)]
                    products(1 - p, 4 * r + n, ties)

    conv_step(0, 0, True, False, False)
    q_cp.start()
    w1_cp.start()
    conv_step(1, 1, True, True, False)
    w2_cp.start()
    w3_cp.start()
    w4_cp.start()

    def conv_pair(it, carry):
        conv_step(2 * it, 0, True, True, True)
        conv_step(2 * it + 1, 1, True, True, True)
        return carry

    lax.fori_loop(1, NCB // 2, conv_pair, 0)
    conv_step(NCB, 0, False, True, True)
    conv_step(NCB + 1, 1, False, False, True)

    def tile(t):
        return _aligned(t * TM, TM)

    def pieces(results, count, lo, hi):
        ps = [r[m * RB:(m + 1) * RB, c:c + 128]
              for r in results for c in range(0, r.shape[1], 128) for m in range(NR)]
        return [ps[int(len(ps) * (lo + (hi - lo) * k / count))] for k in range(count)]

    def after(x, tie):
        if tie is None:
            return x
        return jnp.concatenate([jnp.where(never_rb, tie, x[:, :128]), x[:, 128:]], axis=1)

    def gate(load, r0, along=None, hi=None):
        skew = 2
        ties = pieces(along, NR + 2 * skew, 0.0, hi) if along else [None] * (NR + 2 * skew)
        out = []
        for i in range(NR):
            rows = pl.ds(r0 + i * RB, RB)
            x = after(load(i), ties[i])
            x = x + _ln(x) * xy_s[pl.ds(pl.multiple_of(r0 + i * RB + zero, RB), RB), :]
            z = _ln(after(x, ties[i + skew]))
            xy_s[pl.ds(S + r0 + i * RB, RB), :] = x
            z_s[rows, :] = z
            out.append(_ln(after(z, ties[i + 2 * skew])).astype(bf16))
        return jnp.concatenate(out, axis=0)

    def first_gate(t, along=None):
        r0 = tile(t)
        return gate(lambda i: q_v[pl.ds(r0 + i * RB, RB), :].astype(f32), r0, along, 0.6)

    def token_in(n, r0, h_s):
        res = []
        for j in range(D // NB):
            cols = slice(j * NB, (j + 1) * NB)
            res.append(dot(n, w1_v[:, cols]))
            h_s[pl.ds(r0 + PAD, TM), cols] = _gelu(res[-1])
        return res

    def token_out(r0, h_s):
        c = D // 4
        hv = h_s.at[pl.ds(r0, TM + 2 * PAD), :]
        g = jnp.concatenate([hv[pl.ds(PAD + o, TM), i * c:(i + 1) * c]
                             for i, o in enumerate((-1, 1, -2, 2))], axis=1).astype(bf16)
        res = []
        for j in range(D // NB):
            cols = slice(j * NB, (j + 1) * NB)
            res.append(z_s[pl.ds(r0, TM), cols] + dot(g, w2_v[:, cols]))
            u_s[:, cols] = res[-1]
        return res

    def channel_norm(ties=None):
        for i in range(NR):
            rows = slice(i * RB, (i + 1) * RB)
            n_s[rows, :] = _ln(after(u_s[rows, :], ties[i] if ties else None)).astype(bf16)

    def hidden(n, fc):
        return _gelu(dot(n, w3_v[:, fc * FC:(fc + 1) * FC])).astype(bf16)

    def channel_mlp(n, acc, fcs):
        for fc in fcs:
            acc = acc + dot(hidden(n, fc), w4_v[fc * FC:(fc + 1) * FC, :])
        return acc

    NF = F // FC

    def prologue(t, carry):
        res = token_in(n_s[...], tile(t), h0_s)
        n_s[...] = first_gate(jnp.minimum(t + 1, NT - 1), res)
        return carry

    q_cp.wait()
    n_s[...] = first_gate(0)
    w1_cp.wait()
    lax.fori_loop(0, NT, prologue, 0)
    w2_cp.wait()
    token_out(0, h0_s)
    channel_norm()
    w3_cp.wait()
    w4_cp.wait()

    def layer1(t, carry):
        r0 = tile(t)
        x = channel_mlp(n_s[...], x_s[pl.ds(r0, TM), :] + u_s[...], range(NF))
        res = token_out(tile((t + 1) % NT), h_all.at[(t + 1) // NT])
        n = gate(lambda i: x[i * RB:(i + 1) * RB], r0, res, 0.85)
        res = token_in(n, r0, h1_s)
        channel_norm(pieces(res, NR, 0.05, 0.8))
        return carry

    lax.fori_loop(0, NT, layer1, 0)

    def out_copy(t, cols, sem):
        rows = pl.ds(tile(t), TM)
        return pltpu.make_async_copy(o_v.at[rows, cols], o_hbm.at[rows, cols], osems.at[sem])

    def layer2(t, carry):
        r0 = tile(t)
        n = n_s[...]
        x = channel_mlp(n, x_s[pl.ds(r0, TM), :] + u_s[...], range(NF - 1))
        token_out(tile(t + 1), h1_s)
        x = channel_mlp(n, x, [NF - 1])
        channel_norm()
        o_v[pl.ds(r0, TM), :] = x.astype(bf16)
        out_copy(t, slice(0, D), t).start()
        return carry

    lax.fori_loop(0, NT - 1, layer2, 0)

    t = NT - 1
    n = n_s[...]
    x = channel_mlp(n, x_s[pl.ds(tile(t), TM), :] + u_s[...], range(NF - 1))
    a = hidden(n, NF - 1)
    halves = [slice(0, D // 2), slice(D // 2, D)]
    for j, cols in enumerate(halves):
        o_v[pl.ds(tile(t), TM), cols] = (x[:, cols] + dot(a, w4_v[(NF - 1) * FC:, cols])).astype(bf16)
        out_copy(t, cols, t + j).start()
    for tt in range(NT - 1):
        out_copy(tt, slice(0, D), tt).wait()
    for j, cols in enumerate(halves):
        out_copy(t, cols, t + j).wait()


@jax.jit
def pallas_interleave_layers__ssm_conv_h3__mixer_s_mlp__prompt_kernel(
        A_q, A_k, A_v, A_shift_k, A_ssm_k, A_ssm_D, B_x, B_w1, B_w2, B_w3, B_w4):
    del B_x
    f32, bf16 = jnp.float32, jnp.bfloat16
    hbm = pl.BlockSpec(memory_space=pl.ANY)
    vmem = pl.BlockSpec(memory_space=pltpu.VMEM)
    smem = pl.BlockSpec(memory_space=pltpu.SMEM)
    out = pl.pallas_call(
        _kernel,
        out_shape=jax.ShapeDtypeStruct((S, D), bf16),
        in_specs=[hbm, hbm, hbm, vmem, hbm, vmem, hbm, hbm, hbm, hbm, vmem, vmem, smem],
        out_specs=hbm,
        scratch_shapes=[
            pltpu.VMEM((S, D), bf16),
            pltpu.VMEM((NCB, S, CB), bf16),
            pltpu.VMEM((NCB, S, CB), bf16),
            pltpu.VMEM((NCB, CB, S), bf16),
            pltpu.VMEM((D, D), bf16),
            pltpu.VMEM((D, D), bf16),
            pltpu.VMEM((D, F), bf16),
            pltpu.VMEM((F, D), bf16),
            pltpu.VMEM((S, D), bf16),
            pltpu.VMEM((2 * S, D), f32),
            pltpu.VMEM((S, D), f32),
            pltpu.VMEM((2, S + 2 * PAD, D), f32),
            pltpu.VMEM((TM, D), bf16),
            pltpu.VMEM((TM, D), f32),
            pltpu.VMEM((S + PAD, CB), f32),
            *[pltpu.VMEM((NCH, CB, 3 * C), f32)] * 4,
            *[pltpu.VMEM((NCH, CB, 2 * C), f32)] * 2,
            *[pltpu.VMEM((S, CB), f32)] * 2,
            pltpu.VMEM((NCB, 8, CB), f32),
            pltpu.SemaphoreType.DMA((3 * NCB + 5,)),
            pltpu.SemaphoreType.DMA((NT + 1,)),
        ],
        compiler_params=pltpu.CompilerParams(vmem_limit_bytes=120 * 1024 * 1024),
    )(A_q.reshape(S, D), A_k.reshape(S, D), A_v.reshape(S, D), A_shift_k.T, A_ssm_k, A_ssm_D,
      B_w1, B_w2, B_w3, B_w4, _FWD.astype(bf16), _INV.astype(bf16), np.zeros((1,), np.int32))
    return out.reshape(1, S, D)
```
